```python
import os as _os
_os.environ.setdefault('JAX_PLATFORMS', 'cpu')
import jax
import jax.numpy as jnp

def _softmax(x, axis=-1):
    return jax.nn.softmax(x, axis=axis)

def _gelu(x):
    return jax.nn.gelu(x, approximate=True)

def _silu(x):
    return jax.nn.silu(x)

def _sigmoid(x):
    return jax.nn.sigmoid(x)

def _layernorm(x, axis=-1, eps=1e-05):
    m = jnp.mean(x, axis=axis, keepdims=True)
    v = jnp.var(x, axis=axis, keepdims=True)
    return (x - m) / jnp.sqrt(v + eps)

def _scatter_add(tgt, idx, src, axis=0):
    return tgt.at[idx].add(src)

def _segment_sum(src, seg, n):
    return jax.ops.segment_sum(src, seg, n)

class _Rng:

    def __init__(self, key):
        self._k = key

    def _next(self):
        self._k, sub = jax.random.split(self._k)
        return sub

    def normal(self, shape):
        return jax.random.normal(self._next(), shape, dtype=jnp.bfloat16)

    def randint(self, lo, hi, shape):
        return jax.random.randint(self._next(), shape, lo, hi, dtype=jnp.int32)

    def uniform(self, shape, lo=0.0, hi=1.0):
        return jax.random.uniform(self._next(), shape, jnp.bfloat16, lo, hi)

    def permutation(self, n):
        return jax.random.permutation(self._next(), n)
kernel_name = 'standalone__autoregressive_conv_wavenet__speech'

def setup_inputs():
    _rng = _Rng(jax.random.key(int.from_bytes(__import__("os").urandom(4), "little")))
    _w = lambda a: (lambda t: t.astype(jnp.bfloat16) if jnp.issubdtype(t.dtype, jnp.floating) else t)(jnp.asarray(a))
    B, T, D, K = (2, 4000, 512, 31)
    return {'x': _w((lambda *s: _rng.normal(s) * 0.05)(B, T, D)), 'w': _w((lambda *s: _rng.normal(s) * 0.05)(K, D, 2 * D)), 'w_o': _w((lambda *s: _rng.normal(s) * 0.05)(D, D))}

def reference(x, w, w_o):
    B, T, D = x.shape
    K = w.shape[0]
    dil = 2
    pad = (K - 1) * dil
    xp = jnp.pad(x, ((0, 0), (pad, 0), (0, 0)))
    h = jnp.einsum('btc,cd->btd', xp[:, pad:pad + T, :], w[0])
    for i in range(1, K):
        off = pad - i * dil
        h = h + jnp.einsum('btc,cd->btd', xp[:, off:off + T, :], w[i])
    f = h[..., :D].copy()
    g = h[..., D:].copy()
    z = jnp.tanh(f) * _sigmoid(g)
    return z @ w_o
```

```python
import functools
import numpy as np
import jax
import jax.numpy as jnp
import jax.experimental.pallas as pl
import jax.experimental.pallas.tpu as pltpu


class V:
    __slots__ = ('a', 's')
    def __init__(self, a, s=1):
        self.a = a; self.s = s

def vadd(x, y):
    if x is None: return y
    if y is None: return x
    if x.s == y.s: return V(x.a + y.a, x.s)
    if x.s > 0: return V(x.a - y.a, 1)
    return V(y.a - x.a, 1)
def vneg(x):
    return None if x is None else V(x.a, -x.s)
def vsub(x, y):
    return vadd(x, vneg(y))
def vmul(x, c):
    if x is None: return None
    c = float(c)
    if c == 0.0: return None
    if c == 1.0: return x
    if c == -1.0: return vneg(x)
    return V(x.a * np.float32(c * x.s), 1)
def out(x):
    if x.s > 0: return x.a
    return -x.a

def cadd(x, y): return (vadd(x[0], y[0]), vadd(x[1], y[1]))
def csub(x, y): return (vsub(x[0], y[0]), vsub(x[1], y[1]))
def muli(z, sg):
    return (vneg(z[1]), z[0]) if sg > 0 else (z[1], vneg(z[0]))
def cmul_w(x, k, n, sign=-1):
    k %= n
    if k == 0: return x
    if 4 * k == n: return muli(x, sign)
    if 2 * k == n: return (vneg(x[0]), vneg(x[1]))
    if 4 * k == 3 * n: return muli(x, -sign)
    c = np.cos(2 * np.pi * k / n); s = sign * np.sin(2 * np.pi * k / n)
    if (8 * k) % n == 0:
        r = np.sqrt(0.5)
        sc = c > 0; ss = s > 0
        re = vsub(x[0] if sc else vneg(x[0]), x[1] if ss else vneg(x[1]))
        im = vadd(x[0] if ss else vneg(x[0]), x[1] if sc else vneg(x[1]))
        return (vmul(re, r), vmul(im, r))
    re = vsub(vmul(x[0], c), vmul(x[1], s))
    im = vadd(vmul(x[0], s), vmul(x[1], c))
    return (re, im)

def cfft(x, sign=-1):
    n = len(x)
    if n == 1: return list(x)
    if n == 2: return [cadd(x[0], x[1]), csub(x[0], x[1])]
    h = n // 2; q = n // 4
    s = [cadd(x[t], x[t + h]) for t in range(h)]
    d = [csub(x[t], x[t + h]) for t in range(h)]
    a = [cmul_w(cadd(d[t], muli(d[t + q], sign)), t, n, sign) for t in range(q)]
    b = [cmul_w(csub(d[t], muli(d[t + q], sign)), 3 * t, n, sign) for t in range(q)]
    E = cfft(s, sign); A = cfft(a, sign); B = cfft(b, sign)
    X = [None] * n
    for k in range(h): X[2 * k] = E[k]
    for k in range(q):
        X[4 * k + 1] = A[k]; X[4 * k + 3] = B[k]
    return X


def ON(x):
    return out(x)

def fwd_odd64_bins(C, r):
    res=[]
    for ka in range(4):
        f=4*(r+4*ka)+1
        re,im=C[ka]
        if f<=32: res += [(f,0,re),(f,1,im)]
        else: res += [(64-f,0,re),(64-f,1,vneg(im))]
    return res

def fwd_pass1(lo, hi, u):
    b=[cmul_w((lo[v], vneg(hi[v])), v, 16) for v in range(4)]
    G=cfft(b)
    return [cmul_w(G[r], u*(1+4*r), 64) for r in range(4)]

def rfft_odd(d, n):
    h=n//2; q=n//4; X={}
    if n==2:
        X[1]=(d[0],None); return X
    c=[cmul_w((d[t], vneg(d[t+q])), t, n) for t in range(q)]
    C=cfft(c)
    for k in range(q):
        f=4*k+1
        if f<=h: X[f]=C[k]
        else: X[n-f]=(C[k][0], vneg(C[k][1]))
    return X

def rfft_sc(a):
    n=len(a); h=n//2
    if n==2: return {'sc':(a[0],a[1])}
    s=[vadd(a[t],a[t+h]) for t in range(h)]
    d=[vsub(a[t],a[t+h]) for t in range(h)]
    X={}
    for k,v in rfft_sc(s).items(): X[k if k=='sc' else 2*k]=v
    X.update(rfft_odd(d,n))
    return X

def irfft_odd(Y, n):
    h=n//2; q=n//4
    C=[]
    for k in range(q):
        f=4*k+1
        C.append(Y[f] if f<=h else (Y[n-f][0], vneg(Y[n-f][1])))
    c=cfft(C,+1)
    o=[None]*h
    for t in range(q):
        z=cmul_w(c[t],t,n,+1)
        o[t]=z[0]; o[t+q]=vneg(z[1])
    return o

def irfft_sc(Y, n):
    if n==2: return [Y['sc'][0], Y['sc'][1]]
    h=n//2
    Ye={'sc':Y['sc']}
    for k in range(1,h//2): Ye[k]=Y[2*k]
    e=irfft_sc(Ye,h); o=irfft_odd(Y,n)
    return [vadd(e[t],o[t]) for t in range(h)]+[vsub(e[t],o[t]) for t in range(h)]

def comp_F1(u, ld_in, st_tmp, padded):
    lo=[];hi=[]
    for v in range(4):
        t=u+4*v
        if padded:
            a0=ld_in(t); a1=ld_in(t+16)
            dlo,dhi,slo,shi=a0,a1,a0,a1
        else:
            w0,w1,w2,w3=ld_in(t),ld_in(t+16),ld_in(t+32),ld_in(t+48)
            dlo=vsub(w0,w2); dhi=vsub(w1,w3); slo=vadd(w0,w2); shi=vadd(w1,w3)
        lo.append(dlo); hi.append(dhi)
        st_tmp(32+t, ON(vsub(slo,shi)))
        st_tmp(48+t, ON(vadd(slo,shi)))
    H=fwd_pass1(lo,hi,u)
    for r in range(4):
        st_tmp(u*8+r*2, ON(H[r][0])); st_tmp(u*8+r*2+1, ON(H[r][1]))

def comp_F2(rp, ld_tmp, st_out):
    for r in (2*rp,2*rp+1):
        Hs=[(V(ld_tmp(u*8+r*2)),V(ld_tmp(u*8+r*2+1))) for u in range(4)]
        C=cfft(Hs)
        for (f,p,v) in fwd_odd64_bins(C,r): st_out(f,p,ON(v))

def comp_F3(ld_tmp, st_out):
    d=[V(ld_tmp(32+t)) for t in range(16)]
    X=rfft_odd(d,32)
    for f2,(re,im) in X.items():
        st_out(2*f2,0,ON(re)); st_out(2*f2,1,ON(im))

def comp_F4(ld_tmp, st_out):
    s=[V(ld_tmp(48+t)) for t in range(16)]
    X=rfft_sc(s)
    for k,(re,im) in X.items():
        f=0 if k=='sc' else 4*k
        st_out(f,0,ON(re)); st_out(f,1,ON(im))

def ldY64(ld_y, f):
    if f<=32: return (V(ld_y(f,0)),V(ld_y(f,1)))
    return (V(ld_y(64-f,0)), vneg(V(ld_y(64-f,1))))

def comp_I1(rp, ld_y, st_tmp):
    for r in (2*rp,2*rp+1):
        C=[ldY64(ld_y,4*(r+4*ka)+1) for ka in range(4)]
        G=cfft(C,+1)
        for u in range(4):
            z=cmul_w(G[u],u*(1+4*r),64,+1)
            st_tmp(r*8+u*2,ON(z[0])); st_tmp(r*8+u*2+1,ON(z[1]))

def comp_I2(ld_y, st_tmp):
    Y={f2:(V(ld_y(2*f2,0)),V(ld_y(2*f2,1))) for f2 in range(1,16,2)}
    o=irfft_odd(Y,32)
    for t in range(16): st_tmp(32+t,ON(o[t]))

def comp_I3(ld_y, st_tmp):
    Y={k:(V(ld_y(4*k,0)),V(ld_y(4*k,1))) for k in range(1,8)}
    Y['sc']=(V(ld_y(0,0)),V(ld_y(0,1)))
    e=irfft_sc(Y,16)
    for t in range(16): st_tmp(48+t,ON(e[t]))

def comp_I4(u, ld_tmp, emit):
    G=[(V(ld_tmp(r*8+u*2)),V(ld_tmp(r*8+u*2+1))) for r in range(4)]
    c=cfft(G,+1)
    for v in range(4):
        z=cmul_w(c[v],v,16,+1)
        t=u+4*v
        ee=V(ld_tmp(48+t)); oo=V(ld_tmp(32+t))
        for (tt,e,o) in ((t,vadd(ee,oo),z[0]),(t+16,vsub(ee,oo),vneg(z[1]))):
            emit(tt+2, vsub(e,o))
            if tt>=30: emit(tt-30, vadd(e,o))

F32 = jnp.float32
BF16 = jnp.bfloat16
U32 = jnp.uint32

import contextlib
SCOPES = False
def scope(n):
    return jax.named_scope(n) if SCOPES else contextlib.nullcontext()
MODE = 'ov'

HOP = 34
NBLK = 60
R = 240
XR = 4112
YP = 264
RAWP = 264
Y_OFF = (0, 64 * YP)
RAW_OFF = (2 * 64 * YP, 2 * 64 * YP + 31 * RAWP)
BR = RAW_OFF[1] + 31 * RAWP
TMP_OFF = 0
TMP_W, TMP_I = 0, 4 * 64 * 8
TMP_ANCHOR = 6 * 64 * 8
T_OFF = 0
ZR = 16 * HOP * 16


def ds8(x):
    return pl.ds(pl.multiple_of(x, 8), 8)


def _kernel(offs, x_hbm, w_hbm, wo_hbm, o_hbm, xs, U, whA, whB, big, zb, wo, tmp, Tb, sems):
    whs = (whA, whB)
    bigb = big.bitcast(BF16)
    xsb = xs.bitcast(BF16)

    def off(k, mult=8):
        return pl.multiple_of(offs[k], 8)

    def raw_copies(tile, buf):
        col = (tile % 2) * 512 + (tile // 2) * 128
        if isinstance(col, int):
            cs = pl.ds(col, 128)
        else:
            cs = pl.ds(pl.multiple_of(col, 128), 128)
        return [pltpu.make_async_copy(w_hbm.at[i, :, cs],
                                      bigb.at[pl.ds(2 * (RAW_OFF[buf] + i * RAWP), 512), :],
                                      sems.at[1 + buf]) for i in range(31)]

    x_copies = [pltpu.make_async_copy(x_hbm.at[b, :, pl.ds(ct * 128, 128)],
                                      xsb.at[ct, pl.ds(64 + 4080 * b, 4000), :], sems.at[0])
                for b in range(2) for ct in range(4)]
    wo_copies = [pltpu.make_async_copy(wo_hbm.at[:, pl.ds(nt * 128, 128)], wo.at[nt], sems.at[3]) for nt in range(4)]
    for c in x_copies: c.start()
    for c in raw_copies(0, 0): c.start()
    for c in raw_copies(1, 1): c.start()
    for c in wo_copies: c.start()

    for ct in range(4):
        xs[ct, 0:32, :] = jnp.zeros((32, 128), U32)
        xs[ct, 2032:2072, :] = jnp.zeros((40, 128), U32)
        xs[ct, 4072:4112, :] = jnp.zeros((40, 128), U32)
    def zero_y(p, _):
        for b in range(2):
            big[pl.ds(pl.multiple_of(Y_OFF[b] + p * YP + R, 8), 16), :] = jnp.zeros((16, 128), F32)
        return 0
    jax.lax.fori_loop(0, 64, zero_y, 0)

    with scope('xwait'):
        for c in x_copies: c.wait()

    def x_comps(g, ct, h, tmpb):
        p1, p2 = [], []
        def ld_in(n):
            v = xs[ct, pl.ds(272 * g + 2 + n, 8, stride=HOP), :]
            return V(pltpu.bitcast(v, BF16).astype(F32)[8 * h:8 * h + 8])
        def st_tmp(k, v): tmp[pl.ds(tmpb + k * 8, 8), :] = v
        def ld_tmp(k): return tmp[pl.ds(tmpb + k * 8, 8), :]
        def st_out(f, p, v): U[f, ct, ds8(p * R + 16 * g + 8 * h), :] = v.astype(BF16)
        for u in range(4): p1.append(functools.partial(comp_F1, u, ld_in, st_tmp, False))
        for rp in range(2): p2.append(functools.partial(comp_F2, rp, ld_tmp, st_out))
        p2.append(functools.partial(comp_F3, ld_tmp, st_out))
        p2.append(functools.partial(comp_F4, ld_tmp, st_out))
        return p1, p2

    def w_comps(grp, h, rawb, tmpb, wh):
        p1, p2 = [], []
        def ld_in(t):
            if t >= 31: return None
            v = big[ds8(rawb + RAWP * t + 8 * grp), :]
            return V(pltpu.bitcast(v, BF16).astype(F32)[8 * h:8 * h + 8])
        def st_tmp(k, v): tmp[pl.ds(tmpb + k * 8, 8), :] = v
        def ld_tmp(k): return tmp[pl.ds(tmpb + k * 8, 8), :]
        def st_out(f, p, v): wh[2 * f + p, ds8(16 * grp + 8 * h), :] = v.astype(BF16)
        for u in range(4): p1.append(functools.partial(comp_F1, u, ld_in, st_tmp, True))
        for rp in range(2): p2.append(functools.partial(comp_F2, rp, ld_tmp, st_out))
        p2.append(functools.partial(comp_F3, ld_tmp, st_out))
        p2.append(functools.partial(comp_F4, ld_tmp, st_out))
        return p1, p2

    def inv_comps(kind, g, h, kt, yb, tb, tmpb):
        p1, p2 = [], []
        r0 = 16 * g + 8 * h
        def ld_y(f, p): return big[ds8(yb + (2 * f + p) * YP + r0), :]
        def st_tmp(k, v): tmp[pl.ds(tmpb + k * 8, 8), :] = v
        def ld_tmp(k): return tmp[pl.ds(tmpb + k * 8, 8), :]
        def emit(t, y):
            a = y.a * np.float32(y.s / 32.0)
            if kind == 'f':
                Tb[ds8(t * YP + r0), :] = jnp.tanh(a)
            else:
                z = Tb[ds8(t * YP + r0), :] * jax.nn.sigmoid(a)
                zb[kt, ds8((g * HOP + t) * 16 + 8 * h), :] = z.astype(BF16)
        for rp in range(2): p1.append(functools.partial(comp_I1, rp, ld_y, st_tmp))
        p1.append(functools.partial(comp_I2, ld_y, st_tmp))
        p1.append(functools.partial(comp_I3, ld_y, st_tmp))
        for u in range(4): p2.append(functools.partial(comp_I4, u, ld_tmp, emit))
        return p1, p2

    def interleave(lists):
        res = []
        n = max(len(l) for l in lists) if lists else 0
        pos = [0] * len(lists)
        total = sum(len(l) for l in lists)
        for k in range(total):
            j = min((j for j in range(len(lists)) if pos[j] < len(lists[j])), key=lambda j: (pos[j] + 0.5) / len(lists[j]))
            res.append(lists[j][pos[j]]); pos[j] += 1
        return res

    def xfft_body(i, _):
        g = i // 4; ct = i % 4
        P1, P2 = [], []
        for h in range(2):
            a, b = x_comps(g, ct, h, TMP_OFF + h * 512)
            P1 += a; P2 += b
        for c in P1 + P2: c()
        return 0
    with scope('xfft'):
        jax.lax.fori_loop(0, 60, xfft_body, 0)

    for c in raw_copies(0, 0): c.wait()
    def wfft_body(i, _, buf, wh):
        P1, P2 = [], []
        for lp in range(4):
            a, b = w_comps(2 * i + lp // 2, lp % 2, RAW_OFF[buf], TMP_W + lp * 512, wh)
            P1 += a; P2 += b
        for c in P1 + P2: c()
        return 0
    with scope('wfft0'):
        jax.lax.fori_loop(0, 16, functools.partial(wfft_body, buf=0, wh=whA), 0)

    def inv_body(i, _, kind, kt, yoff):
        P1, P2 = [], []
        for h in range(2):
            a, b = inv_comps(kind, i, h, kt, yoff, T_OFF, TMP_I + h * 512)
            P1 += a; P2 += b
        for c in P1 + P2: c()
        return 0

    def step(par, has_w, inv_kind, s, next_dma):
        wh_cur, wh_nxt = whs[par], whs[1 - par]
        if has_w:
            for c in raw_copies(s + 1, 1 - par): c.wait()
        if next_dma:
            for c in raw_copies(s + 2, par): c.start()
        kt_prev = (s - 1) // 2

        def body(i, _):
            ycur = off(0) + Y_OFF[par] + i * (4 * YP)
            streams = []
            if MODE == 'ov':
                if has_w:
                    rawb = off(2) + RAW_OFF[1 - par]
                    g1, g2 = [], []
                    for lp in range(4):
                        a, b = w_comps(2 * i + lp // 2, lp % 2, rawb, TMP_W + lp * 512, wh_nxt)
                        g1.append([(1, c) for c in a]); g2.append([(2, c) for c in b])
                    streams.append(g1[0] + g1[1] + g2[0] + g1[2] + g2[1] + g1[3] + g2[2] + g2[3])
                if inv_kind:
                    yprev = off(1) + Y_OFF[1 - par]
                    g1, g2 = [], []
                    for h in range(2):
                        a, b = inv_comps(inv_kind, i, h, kt_prev, yprev, 0, TMP_I + h * 512)
                        g1.append([(1, c) for c in a]); g2.append([(2, c) for c in b])
                    streams.append(g1[0] + g1[1] + g2[0] + g2[1])
            cl = interleave(streams)
            nan = 120
            slots = {}
            for k, c in enumerate(cl):
                slots.setdefault((k * nan) // max(len(cl), 1), []).append(c)
            anchor_at = pl.ds(off(3) + TMP_ANCHOR, 8)
            def run_slot(k, piece):
                for kind, c in slots.get(k, []):
                    if kind == 2:
                        tmp[anchor_at, :] = piece
                    c()
            ak = 0
            for qq in range(2):
                q = 2 * i + qq
                lhs = jnp.concatenate([U[q, kt] for kt in range(4)], axis=1)
                yr = ycur + (2 * qq) * YP
                yi = ycur + (2 * qq + 1) * YP
                P = jnp.dot(lhs, wh_cur[2 * q], preferred_element_type=F32)
                PIECE = P
                for g in range(30):
                    dst = (yr if g < 15 else yi) + 16 * (g % 15)
                    big[pl.ds(pl.multiple_of(dst, 8), 16), :] = P[16 * g:16 * g + 16]
                    run_slot(ak, PIECE[16 * g:16 * g + 8])
                    ak += 1
                Q = jnp.dot(lhs, wh_cur[2 * q + 1], preferred_element_type=F32)
                PIECE = Q
                if qq == 0:
                    sigma = jnp.where(i == 0, 1.0, -1.0).astype(F32)
                for g in range(30):
                    dst = (yi if g < 15 else yr) + 16 * (g % 15)
                    d = pl.ds(pl.multiple_of(dst, 8), 16)
                    if g < 15:
                        big[d, :] = big[d, :] + Q[16 * g:16 * g + 16]
                    elif qq == 0:
                        big[d, :] = big[d, :] + sigma * Q[16 * g:16 * g + 16]
                    else:
                        big[d, :] = big[d, :] - Q[16 * g:16 * g + 16]
                    run_slot(ak, PIECE[16 * g:16 * g + 8])
                    ak += 1
            return 0
        jax.lax.fori_loop(0, 16, body, 0)
        if MODE == 'seq':
            if has_w:
                jax.lax.fori_loop(0, 16, functools.partial(wfft_body, buf=1 - par, wh=wh_nxt), 0)
            if inv_kind:
                jax.lax.fori_loop(0, 16, functools.partial(inv_body, kind=inv_kind, kt=kt_prev, yoff=Y_OFF[1 - par]), 0)

    with scope('step0'):
        step(0, True, None, 0, True)
    if True:
        def pair_body(qp, _):
            s = 2 * qp + 1
            step_dyn(1, 'f', s)
            step_dyn(0, 'g', s + 1)
            return 0

        def step_dyn(par, kind, s):
            @pl.when(s + 2 <= 7)
            def _():
                for c in raw_copies(s + 2, par): c.start()
            step(par, True, kind, s, False)
        with scope('steps16'):
            jax.lax.fori_loop(0, 3, pair_body, 0)
    with scope('step7'):
        step(1, False, 'f', 7, False)

    with scope('inv7'):
        jax.lax.fori_loop(0, 15, functools.partial(inv_body, kind='g', kt=3, yoff=Y_OFF[1]), 0)

    for c in wo_copies: c.wait()

    def out_copy(row0, nrows, b, orow0, nt):
        return pltpu.make_async_copy(xsb.at[nt, pl.ds(row0, nrows), :],
                                     o_hbm.at[b, pl.ds(orow0, nrows), pl.ds(nt * 128, 128)], sems.at[4])
    def pieces(g):
        if g < 7: return [(544 * g, 544, 0, 544 * g)]
        if g == 7: return [(3808, 192, 0, 3808), (4080, 272, 1, 0)]
        if g < 14: return [(544 * g, 544, 1, 544 * g - 4080)]
        return [(544 * 14, 464, 1, 544 * 14 - 4080)]

    def fin_body(g, _):
        lhs = jnp.concatenate([zb[kt, pl.ds(pl.multiple_of(g * 544, 16), 544), :] for kt in range(4)], axis=1)
        for nt in range(4):
            Rr = jnp.dot(lhs, wo[nt], preferred_element_type=F32)
            for t in range(HOP):
                v = pltpu.bitcast(Rr[16 * t:16 * t + 16].astype(BF16), U32)
                xs[nt, pl.ds(272 * g + t, 8, stride=HOP), :] = v
        @pl.when(g < 7)
        def _():
            for nt in range(4):
                out_copy(pl.multiple_of(544 * g, 16), 544, 0, pl.multiple_of(544 * g, 16), nt).start()
        @pl.when(g == 7)
        def _():
            for nt in range(4):
                for (a, n, b, o) in pieces(7): out_copy(a, n, b, o, nt).start()
        @pl.when((g > 7) & (g < 14))
        def _():
            for nt in range(4):
                out_copy(pl.multiple_of(544 * g, 16), 544, 1, pl.multiple_of(544 * g - 4080, 16), nt).start()
        @pl.when(g == 14)
        def _():
            for nt in range(4):
                for (a, n, b, o) in pieces(14): out_copy(a, n, b, o, nt).start()
        return 0
    with scope('final'):
        jax.lax.fori_loop(0, 15, fin_body, 0)
    for g in range(15):
        for nt in range(4):
            for (a, n, b, o) in pieces(g): out_copy(a, n, b, o, nt).wait()


@jax.jit
def pallas_standalone__autoregressive_conv_wavenet__speech_kernel(x, w, w_o):
    B, T, D = x.shape
    offs = jnp.asarray(np.zeros((8,), np.int32))
    return pl.pallas_call(
        _kernel,
        in_specs=[pl.BlockSpec(memory_space=pltpu.SMEM)] + [pl.BlockSpec(memory_space=pl.ANY)] * 3,
        out_specs=pl.BlockSpec(memory_space=pl.ANY),
        out_shape=jax.ShapeDtypeStruct((B, T, D), x.dtype),
        scratch_shapes=[
            pltpu.VMEM((4, XR, 128), U32),
            pltpu.VMEM((32, 4, 2 * R, 128), BF16),
            pltpu.VMEM((64, 512, 128), BF16),
            pltpu.VMEM((64, 512, 128), BF16),
            pltpu.VMEM((BR, 128), F32),
            pltpu.VMEM((4, ZR, 128), BF16),
            pltpu.VMEM((4, 512, 128), BF16),
            pltpu.VMEM((6 * 64 * 8 + 8, 128), F32),
            pltpu.VMEM((34 * YP, 128), F32),
            pltpu.SemaphoreType.DMA((5,)),
        ],
        compiler_params=pltpu.CompilerParams(vmem_limit_bytes=120 * 1024 * 1024),
    )(offs, x, w, w_o)
```

```python
import functools
import numpy as np
import jax
import jax.numpy as jnp
import jax.experimental.pallas as pl
import jax.experimental.pallas.tpu as pltpu

import contextlib
SCOPES = False
def scope(n):
    return jax.named_scope(n) if SCOPES else contextlib.nullcontext()


class V:
    __slots__ = ('a', 's')
    def __init__(self, a, s=1):
        self.a = a; self.s = s

def vadd(x, y):
    if x is None: return y
    if y is None: return x
    if x.s == y.s: return V(x.a + y.a, x.s)
    if x.s > 0: return V(x.a - y.a, 1)
    return V(y.a - x.a, 1)
def vneg(x):
    return None if x is None else V(x.a, -x.s)
def vsub(x, y):
    return vadd(x, vneg(y))
def vmul(x, c):
    if x is None: return None
    c = float(c)
    if c == 0.0: return None
    if c == 1.0: return x
    if c == -1.0: return vneg(x)
    return V(x.a * np.float32(c * x.s), 1)
def out(x):
    if x.s > 0: return x.a
    return -x.a

def cadd(x, y): return (vadd(x[0], y[0]), vadd(x[1], y[1]))
def csub(x, y): return (vsub(x[0], y[0]), vsub(x[1], y[1]))
def muli(z, sg):
    return (vneg(z[1]), z[0]) if sg > 0 else (z[1], vneg(z[0]))
def cmul_w(x, k, n, sign=-1):
    k %= n
    if k == 0: return x
    if 4 * k == n: return muli(x, sign)
    if 2 * k == n: return (vneg(x[0]), vneg(x[1]))
    if 4 * k == 3 * n: return muli(x, -sign)
    c = np.cos(2 * np.pi * k / n); s = sign * np.sin(2 * np.pi * k / n)
    if (8 * k) % n == 0:
        r = np.sqrt(0.5)
        sc = c > 0; ss = s > 0
        re = vsub(x[0] if sc else vneg(x[0]), x[1] if ss else vneg(x[1]))
        im = vadd(x[0] if ss else vneg(x[0]), x[1] if sc else vneg(x[1]))
        return (vmul(re, r), vmul(im, r))
    re = vsub(vmul(x[0], c), vmul(x[1], s))
    im = vadd(vmul(x[0], s), vmul(x[1], c))
    return (re, im)

def cfft(x, sign=-1):
    n = len(x)
    if n == 1: return list(x)
    if n == 2: return [cadd(x[0], x[1]), csub(x[0], x[1])]
    h = n // 2; q = n // 4
    s = [cadd(x[t], x[t + h]) for t in range(h)]
    d = [csub(x[t], x[t + h]) for t in range(h)]
    a = [cmul_w(cadd(d[t], muli(d[t + q], sign)), t, n, sign) for t in range(q)]
    b = [cmul_w(csub(d[t], muli(d[t + q], sign)), 3 * t, n, sign) for t in range(q)]
    E = cfft(s, sign); A = cfft(a, sign); B = cfft(b, sign)
    X = [None] * n
    for k in range(h): X[2 * k] = E[k]
    for k in range(q):
        X[4 * k + 1] = A[k]; X[4 * k + 3] = B[k]
    return X


def rfft_odd(d, n):
    h=n//2; q=n//4; X={}
    if n==2:
        X[1]=(d[0],None); return X
    c=[cmul_w((d[t], vneg(d[t+q])), t, n) for t in range(q)]
    C=cfft(c)
    for k in range(q):
        f=4*k+1
        if f<=h: X[f]=C[k]
        else: X[n-f]=(C[k][0], vneg(C[k][1]))
    return X

def rfft(a):
    n=len(a); h=n//2
    if n==1: return {0:(a[0],None)}
    s=[vadd(a[t],a[t+h]) for t in range(h)]
    d=[vsub(a[t],a[t+h]) for t in range(h)]
    X={2*k:v for k,v in rfft(s).items()}
    X.update(rfft_odd(d,n))
    return X

def irfft_odd(Y, n):
    h=n//2; q=n//4
    if n==2: return [Y[1][0]]
    C=[]
    for k in range(q):
        f=4*k+1
        C.append(Y[f] if f<=h else (Y[n-f][0], vneg(Y[n-f][1])))
    c=cfft(C,+1)
    o=[None]*h
    for t in range(q):
        z=cmul_w(c[t],t,n,+1)
        o[t]=z[0]; o[t+q]=vneg(z[1])
    return o

def irfft_eo(Y, n):
    h=n//2
    if h==1: e=[Y[0][0]]
    else:
        ee,oo=irfft_eo({k:Y[2*k] for k in range(h//2+1)},h)
        e=[vadd(ee[t],oo[t]) for t in range(h//2)]+[vsub(ee[t],oo[t]) for t in range(h//2)]
    return e, irfft_odd(Y,n)

def comp_F1(u, ld_in, st_tmp):
    X=rfft([ld_in(u+4*v) for v in range(16)])
    for f in range(1,8):
        z=cmul_w(X[f],u*f,64)
        st_tmp((f-1)*8+2*u, out(z[0])); st_tmp((f-1)*8+2*u+1, out(z[1]))
    st_tmp(56+u, out(X[0][0])); st_tmp(60+u, out(X[8][0]))

def comp_F2(fs, ld_tmp, st_out):
    for f in fs:
        if f==0:
            r=[V(ld_tmp(56+u)) for u in range(4)]
            st_out(0, vadd(r[0],r[2]), vadd(r[1],r[3]))
            st_out(16, vsub(r[0],r[2]), vsub(r[3],r[1]))
            s=[V(ld_tmp(60+u)) for u in range(4)]
            h=np.sqrt(0.5)
            dm=vmul(vsub(s[1],s[3]),h); sm=vmul(vadd(s[1],s[3]),h)
            st_out(8, vadd(s[0],dm), vneg(vadd(s[2],sm)))
            st_out(24, vsub(s[0],dm), vsub(s[2],sm))
        else:
            T=[(V(ld_tmp((f-1)*8+2*u)),V(ld_tmp((f-1)*8+2*u+1))) for u in range(4)]
            C=cfft(T)
            for (b,z,cj) in ((f,C[0],False),(16+f,C[1],False),(32-f,C[2],True),(16-f,C[3],True)):
                st_out(b, z[0], vneg(z[1]) if cj else z[1])

def comp_I1(fs, ld_y, st_tmp):
    for f in fs:
        if f==0:
            yr,yi=V(ld_y(0,0)),V(ld_y(0,1))
            a,b=V(ld_y(16,0)),V(ld_y(16,1))
            for u,v in enumerate((vadd(yr,a),vsub(yi,b),vsub(yr,a),vadd(yi,b))): st_tmp(56+u,out(v))
            Y8=(V(ld_y(8,0)),V(ld_y(8,1))); Y24=(V(ld_y(24,0)),V(ld_y(24,1)))
            h=np.sqrt(0.5)
            p=vsub(Y8[0],Y24[0]); q=vadd(Y8[1],Y24[1])
            p2=vadd(Y8[0],Y24[0]); q2=vsub(Y24[1],Y8[1])
            z0=p2
            z1=vmul(vsub(p,q),h)
            z2=q2
            z3=vmul(vneg(vadd(p,q)),h)
            for u,v in enumerate((z0,z1,z2,z3)): st_tmp(60+u,out(v))
        else:
            def Y(F):
                if F<=32: return (V(ld_y(F,0)),V(ld_y(F,1)))
                return (V(ld_y(64-F,0)),vneg(V(ld_y(64-F,1))))
            G=cfft([Y(f),Y(f+16),Y(f+32),Y(f+48)],+1)
            for u in range(4):
                z=cmul_w(G[u],u*f,64,+1)
                st_tmp((f-1)*8+2*u,out(z[0])); st_tmp((f-1)*8+2*u+1,out(z[1]))

def comp_I2(u, ld_tmp, emit):
    Z={f:(V(ld_tmp((f-1)*8+2*u)),V(ld_tmp((f-1)*8+2*u+1))) for f in range(1,8)}
    Z[0]=(V(ld_tmp(56+u)),None); Z[8]=(V(ld_tmp(60+u)),None)
    e,o=irfft_eo(Z,16)
    for v in range(8):
        emit(u+4*(v+8)-30, vsub(e[v],o[v]))
    if u>=2: emit(u+28-30, vadd(e[7],o[7]))

F32 = jnp.float32
BF16 = jnp.bfloat16
U32 = jnp.uint32

FGROUPS = ((0, 1), (2, 3), (4, 5), (6, 7))
TAILGAP = 6
UNROLL = 2
HOP = 34
R = 240
XR = 4112
YP = 264
RAWP = 264
Y_OFF = (0, 64 * YP)
RAW_OFF = (2 * 64 * YP, 2 * 64 * YP + 31 * RAWP)
ANCH_OFF = RAW_OFF[1] + 32 * RAWP
BR = ANCH_OFF + 8
TMP_ANCHOR = 3 * 1024 * UNROLL
ZW = 16 * HOP * 8
ZR = 2 * ZW


def tap_slot(t):
    return (t % 4) * 8 + t // 4


def ds8(x, n=8):
    return pl.ds(pl.multiple_of(x, 8), n)


def interleave(lists):
    res = []
    pos = [0] * len(lists)
    total = sum(len(l) for l in lists)
    for _ in range(total):
        j = min((j for j in range(len(lists)) if pos[j] < len(lists[j])),
                key=lambda j: (pos[j] + 0.5) / len(lists[j]))
        res.append(lists[j][pos[j]]); pos[j] += 1
    return res


def pack16(v):
    return pltpu.bitcast(v.astype(BF16), U32)


def _kernel(offs, x_hbm, w_hbm, wo_hbm, o_hbm, xs, U, whA, whB, big, zb, wo, tmp, Tb, sems, xsems):
    whs = (whA, whB)
    bigb = big.bitcast(BF16)
    xsb = xs.bitcast(BF16)
    Uw = U.bitcast(U32)
    whw = (whA.bitcast(U32), whB.bitcast(U32))
    zw = zb.bitcast(U32)
    wow = wo.bitcast(U32)

    def off(k):
        return pl.multiple_of(offs[k], 8)

    def raw_copies(tile, buf):
        col = (tile % 2) * 512 + (tile // 2) * 128
        cs = pl.ds(col, 128) if isinstance(col, int) else pl.ds(pl.multiple_of(col, 128), 128)
        return [pltpu.make_async_copy(w_hbm.at[i, :, cs],
                                      bigb.at[pl.ds(2 * (RAW_OFF[buf] + tap_slot(i) * RAWP), 512), :],
                                      sems.at[1 + buf]) for i in range(31)]

    def x_copy(b, ct):
        cs = pl.ds(ct * 128, 128) if isinstance(ct, int) else pl.ds(pl.multiple_of(ct * 128, 128), 128)
        return pltpu.make_async_copy(x_hbm.at[b, :, cs],
                                     xsb.at[ct, pl.ds(64 + 4080 * b, 4000), :], xsems.at[ct * 2 + b])
    wo_copies = [pltpu.make_async_copy(wo_hbm.at[:, pl.ds(nt * 128, 128)], wo.at[nt], sems.at[3]) for nt in range(4)]
    x_copy(0, 0).start()
    x_copy(1, 0).start()

    for ct in range(4):
        xs[ct, 0:32, :] = jnp.zeros((32, 128), U32)
        xs[ct, 2032:2072, :] = jnp.zeros((40, 128), U32)
        xs[ct, 4072:4112, :] = jnp.zeros((40, 128), U32)
    def zero_y(p, _):
        for b in range(2):
            big[ds8(Y_OFF[b] + p * YP + R, 16), :] = jnp.zeros((16, 128), F32)
        return 0
    jax.lax.fori_loop(0, 64, zero_y, 0)

    def fwd_comps(ld_word, padded, tmpb, st_out):
        p1, p2 = [], []
        for h in range(2):
            def ld_in(n, h=h):
                if padded and n >= 31: return None
                return V(pltpu.bitcast(ld_word(n), BF16).astype(F32)[8 * h:8 * h + 8])
            def st_tmp(k, v, h=h): tmp[ds8(tmpb + k * 16 + 8 * h), :] = v
            p1.append([functools.partial(comp_F1, u, ld_in, st_tmp) for u in range(4)])
        def ld_tmp(k): return tmp[ds8(tmpb + k * 16, 16), :]
        for fs in FGROUPS:
            p2.append(functools.partial(comp_F2, fs, ld_tmp, st_out))
        return p1, p2

    def x_comps(g, ct, tmpb):
        def ld_word(n): return xs[ct, pl.ds(272 * g + 2 + n, 8, stride=HOP), :]
        def st_out(f, re, im):
            planes = (re, vsub(re, im) if f == 0 else vadd(re, im), vsub(im, re))
            for p, v in enumerate(planes):
                U[f, ct, pl.ds(pl.multiple_of(p * R + 16 * g, 16), 16), :] = out(v).astype(BF16)
        return fwd_comps(ld_word, False, tmpb, st_out)

    def w_comps(grp, rawb, tmpb, wh):
        def ld_word(t): return big[ds8(rawb + RAWP * tap_slot(t) + 8 * grp), :]
        def st_out(f, re, im):
            for p, v in enumerate((vadd(re, im), im, re)):
                wh[3 * f + p, pl.ds(pl.multiple_of(16 * grp, 16), 16), :] = out(v).astype(BF16)
        return fwd_comps(ld_word, True, tmpb, st_out)

    def inv_comps(kind, g, zbase, yb, tmpb):
        p1, p2 = [], []
        for h in range(2):
            def ld_y(f, p, h=h): return big[ds8(yb + (2 * f + p) * YP + 16 * g + 8 * h), :]
            def st_tmp(k, v, h=h): tmp[ds8(tmpb + k * 16 + 8 * h), :] = v
            p1.append([functools.partial(comp_I1, fs, ld_y, st_tmp) for fs in FGROUPS])
        for h in range(2):
            def ld_tmp(k, h=h): return tmp[ds8(tmpb + k * 16 + 8 * h), :]
            if kind == 'f':
                def emit(t, y, h=h):
                    Tb[ds8(t * YP + 16 * g + 8 * h), :] = jnp.tanh(y.a * np.float32(y.s / 32.0)) * np.float32(0.5)
            else:
                def emit(t, y, h=h):
                    th = Tb[ds8(t * YP + 16 * g + 8 * h), :]
                    z = th + th * jnp.tanh(y.a * np.float32(y.s / 64.0))
                    zb[ds8(zbase + t * 16 + 8 * h), :] = z.astype(BF16)
            p2.append([functools.partial(comp_I2, u, ld_tmp, emit) for u in range(4)])
        return p1, p2

    def xfft_body(i, _):
        ct = i // 15
        g = i - 15 * ct
        @pl.when(g == 0)
        def _():
            x_copy(0, ct).wait()
            @pl.when(ct < 3)
            def _():
                x_copy(0, ct + 1).start()
            @pl.when(ct == 3)
            def _():
                for c in raw_copies(1, 1): c.start()
                for c in wo_copies: c.start()
        @pl.when(g == 7)
        def _():
            x_copy(1, ct).wait()
            @pl.when(ct < 3)
            def _():
                x_copy(1, ct + 1).start()
            @pl.when(ct == 2)
            def _():
                for c in raw_copies(0, 0): c.start()
        p1, p2 = x_comps(g, ct, 0)
        for c in p1[0] + p1[1] + p2: c()
        return 0
    with scope('xfft'):
        jax.lax.fori_loop(0, 60, xfft_body, 0)

    for c in raw_copies(0, 0): c.wait()
    def wfft_body(i, _):
        P1, P2 = [], []
        for lp in range(2):
            a, b = w_comps(2 * i + lp, RAW_OFF[0], lp * 1024, whA)
            P1 += a[0] + a[1]; P2 += b
        for c in P1 + P2: c()
        return 0
    with scope('wfft0'):
        jax.lax.fori_loop(0, 16, wfft_body, 0)

    def inv_body(i, _):
        zbase = 3 * ZR + i * (HOP * 16)
        p1, p2 = inv_comps('g', i, zbase, Y_OFF[1], 0)
        for c in p1[0] + p1[1] + p2[0] + p2[1]: c()
        return 0

    NIT = 16 // UNROLL
    def step(par, has_w, inv_kind, s):
        wh_cur, wh_nxt = whw[par], whs[1 - par]
        if has_w:
            for c in raw_copies(s + 1, 1 - par): c.wait()
        kt_prev = (s - 1) // 2

        def body(i, _):
            ycur = off(0) + Y_OFF[par] + i * (4 * UNROLL * YP)
            streams = []
            if has_w:
                rawb = off(2) + RAW_OFF[1 - par]
                seq = []
                prev2 = None
                for lp in range(2 * UNROLL):
                    a, b = w_comps(2 * UNROLL * i + lp, rawb, lp * 1024, wh_nxt)
                    seq += [(1, c) for c in a[0]]
                    h2 = [(1, c) for c in a[1]]
                    if prev2:
                        h2 = interleave([h2, prev2])
                    seq += h2
                    prev2 = [(2, c) for c in b]
                seq += prev2
                streams.append(seq)
            if inv_kind:
                yprev = off(1) + Y_OFF[1 - par]
                seq = []
                prev2 = []
                for lp in range(UNROLL):
                    g = UNROLL * i + lp
                    zbase = kt_prev * ZR + g * (HOP * 16)
                    a, b = inv_comps(inv_kind, g, zbase, yprev, (2 * UNROLL + lp) * 1024)
                    seq += interleave([[(1, c) for c in a[0]], prev2])
                    seq += interleave([[(1, c) for c in a[1]], [(2, c) for c in b[0]]])
                    prev2 = [(2, c) for c in b[1]]
                seq += prev2
                streams.append(seq)
            cl = interleave(streams)
            nan = 90 * UNROLL
            slots = {}
            span = nan - TAILGAP
            for k, c in enumerate(cl):
                slots.setdefault((k * span) // max(len(cl), 1), []).append(c)
            anchor_at = pl.ds(off(3) + TMP_ANCHOR, 8)
            def run_slot(k, piece):
                for kind, c in slots.get(k, []):
                    if kind == 2:
                        tmp[anchor_at, :] = piece
                    c()
            ak = 0
            for qq in range(2 * UNROLL):
                q = 2 * UNROLL * i + qq
                yr = ycur + (2 * qq) * YP
                yi = ycur + (2 * qq + 1) * YP
                for m in range(3):
                    lhs = jnp.concatenate([pltpu.bitcast(Uw[q, kt, pl.ds(m * (R // 2), R // 2), :], BF16) for kt in range(4)], axis=1)
                    K = jnp.dot(lhs, pltpu.bitcast(wh_cur[3 * q + m], BF16), preferred_element_type=F32)
                    for g in range(15):
                        piece = K[16 * g:16 * g + 16]
                        di = ds8(yi + 16 * g, 16)
                        if m == 0:
                            big[di, :] = piece
                        elif m == 1:
                            big[ds8(yr + 16 * g, 16), :] = big[di, :] - piece
                        else:
                            big[di, :] = big[di, :] + piece
                        run_slot(ak, piece[:8]); ak += 1
            return 0
        jax.lax.fori_loop(0, NIT, body, 0)

    for c in raw_copies(2, 0): c.start()
    with scope('step0'):
        step(0, True, None, 0)

    def pair_body(qp, _):
        s = 2 * qp + 1
        @pl.when(s + 2 <= 7)
        def _():
            for c in raw_copies(s + 2, 1): c.start()
        step(1, True, 'f', s)
        @pl.when(s + 3 <= 7)
        def _():
            for c in raw_copies(s + 3, 0): c.start()
        step(0, True, 'g', s + 1)
        return 0
    with scope('steps16'):
        jax.lax.fori_loop(0, 3, pair_body, 0)
    with scope('step7'):
        step(1, False, 'f', 7)

    with scope('inv7'):
        jax.lax.fori_loop(0, 15, inv_body, 0)

    for c in wo_copies: c.wait()

    def out_copy(row0, nrows, b, orow0, nt):
        return pltpu.make_async_copy(xsb.at[nt, pl.ds(row0, nrows), :],
                                     o_hbm.at[b, pl.ds(orow0, nrows), pl.ds(nt * 128, 128)], sems.at[4])
    def pieces(g):
        if g < 7: return [(544 * g, 544, 0, 544 * g)]
        if g == 7: return [(3808, 192, 0, 3808), (4080, 272, 1, 0)]
        if g < 14: return [(544 * g, 544, 1, 544 * g - 4080)]
        return [(544 * 14, 464, 1, 544 * 14 - 4080)]

    def fin_body(g, _):
        lhs = jnp.concatenate([pltpu.bitcast(zw[ds8(kt * ZW + g * (HOP * 8), HOP * 8), :], BF16) for kt in range(4)], axis=1)
        for nt in range(4):
            Rr = jnp.dot(lhs, pltpu.bitcast(wow[nt], BF16), preferred_element_type=F32)
            for t in range(HOP):
                xs[nt, pl.ds(272 * g + t, 8, stride=HOP), :] = pack16(Rr[16 * t:16 * t + 16])
        @pl.when(g < 7)
        def _():
            for nt in range(4):
                out_copy(pl.multiple_of(544 * g, 16), 544, 0, pl.multiple_of(544 * g, 16), nt).start()
        @pl.when(g == 7)
        def _():
            for nt in range(4):
                for (a, n, b, o) in pieces(7): out_copy(a, n, b, o, nt).start()
        @pl.when((g > 7) & (g < 14))
        def _():
            for nt in range(4):
                out_copy(pl.multiple_of(544 * g, 16), 544, 1, pl.multiple_of(544 * g - 4080, 16), nt).start()
        @pl.when(g == 14)
        def _():
            for nt in range(4):
                for (a, n, b, o) in pieces(14): out_copy(a, n, b, o, nt).start()
        return 0
    with scope('final'):
        jax.lax.fori_loop(0, 15, fin_body, 0)
    for g in range(15):
        for nt in range(4):
            for (a, n, b, o) in pieces(g): out_copy(a, n, b, o, nt).wait()


@jax.jit
def pallas_standalone__autoregressive_conv_wavenet__speech_kernel(x, w, w_o):
    B, T, D = x.shape
    offs = jnp.asarray(np.zeros((8,), np.int32))
    return pl.pallas_call(
        _kernel,
        in_specs=[pl.BlockSpec(memory_space=pltpu.SMEM)] + [pl.BlockSpec(memory_space=pl.ANY)] * 3,
        out_specs=pl.BlockSpec(memory_space=pl.ANY),
        out_shape=jax.ShapeDtypeStruct((B, T, D), x.dtype),
        scratch_shapes=[
            pltpu.VMEM((4, XR, 128), U32),
            pltpu.VMEM((32, 4, 3 * R, 128), BF16),
            pltpu.VMEM((96, 512, 128), BF16),
            pltpu.VMEM((96, 512, 128), BF16),
            pltpu.VMEM((BR, 128), F32),
            pltpu.VMEM((4 * ZR, 128), BF16),
            pltpu.VMEM((4, 512, 128), BF16),
            pltpu.VMEM((TMP_ANCHOR + 8, 128), F32),
            pltpu.VMEM((34 * YP, 128), F32),
            pltpu.SemaphoreType.DMA((5,)),
            pltpu.SemaphoreType.DMA((8,)),
        ],
        compiler_params=pltpu.CompilerParams(vmem_limit_bytes=120 * 1024 * 1024),
    )(offs, x, w, w_o)
```

```python
import functools
import numpy as np
import jax
import jax.numpy as jnp
import jax.experimental.pallas as pl
import jax.experimental.pallas.tpu as pltpu


class V:
    __slots__ = ('a', 's')
    def __init__(self, a, s=1):
        self.a = a; self.s = s

def vadd(x, y):
    if x is None: return y
    if y is None: return x
    if x.s == y.s: return V(x.a + y.a, x.s)
    if x.s > 0: return V(x.a - y.a, 1)
    return V(y.a - x.a, 1)
def vneg(x):
    return None if x is None else V(x.a, -x.s)
def vsub(x, y):
    return vadd(x, vneg(y))
def vmul(x, c):
    if x is None: return None
    c = float(c)
    if c == 0.0: return None
    if c == 1.0: return x
    if c == -1.0: return vneg(x)
    return V(x.a * np.float32(c * x.s), 1)
def out(x):
    if x.s > 0: return x.a
    return -x.a

def cadd(x, y): return (vadd(x[0], y[0]), vadd(x[1], y[1]))
def csub(x, y): return (vsub(x[0], y[0]), vsub(x[1], y[1]))
def muli(z, sg):
    return (vneg(z[1]), z[0]) if sg > 0 else (z[1], vneg(z[0]))
def cmul_w(x, k, n, sign=-1):
    k %= n
    if k == 0: return x
    if 4 * k == n: return muli(x, sign)
    if 2 * k == n: return (vneg(x[0]), vneg(x[1]))
    if 4 * k == 3 * n: return muli(x, -sign)
    c = np.cos(2 * np.pi * k / n); s = sign * np.sin(2 * np.pi * k / n)
    if (8 * k) % n == 0:
        r = np.sqrt(0.5)
        sc = c > 0; ss = s > 0
        re = vsub(x[0] if sc else vneg(x[0]), x[1] if ss else vneg(x[1]))
        im = vadd(x[0] if ss else vneg(x[0]), x[1] if sc else vneg(x[1]))
        return (vmul(re, r), vmul(im, r))
    re = vsub(vmul(x[0], c), vmul(x[1], s))
    im = vadd(vmul(x[0], s), vmul(x[1], c))
    return (re, im)

def cfft(x, sign=-1):
    n = len(x)
    if n == 1: return list(x)
    if n == 2: return [cadd(x[0], x[1]), csub(x[0], x[1])]
    h = n // 2; q = n // 4
    s = [cadd(x[t], x[t + h]) for t in range(h)]
    d = [csub(x[t], x[t + h]) for t in range(h)]
    a = [cmul_w(cadd(d[t], muli(d[t + q], sign)), t, n, sign) for t in range(q)]
    b = [cmul_w(csub(d[t], muli(d[t + q], sign)), 3 * t, n, sign) for t in range(q)]
    E = cfft(s, sign); A = cfft(a, sign); B = cfft(b, sign)
    X = [None] * n
    for k in range(h): X[2 * k] = E[k]
    for k in range(q):
        X[4 * k + 1] = A[k]; X[4 * k + 3] = B[k]
    return X


def rfft_odd(d, n):
    h=n//2; q=n//4; X={}
    if n==2:
        X[1]=(d[0],None); return X
    c=[cmul_w((d[t], vneg(d[t+q])), t, n) for t in range(q)]
    C=cfft(c)
    for k in range(q):
        f=4*k+1
        if f<=h: X[f]=C[k]
        else: X[n-f]=(C[k][0], vneg(C[k][1]))
    return X

def rfft(a):
    n=len(a); h=n//2
    if n==1: return {0:(a[0],None)}
    s=[vadd(a[t],a[t+h]) for t in range(h)]
    d=[vsub(a[t],a[t+h]) for t in range(h)]
    X={2*k:v for k,v in rfft(s).items()}
    X.update(rfft_odd(d,n))
    return X

def irfft_odd(Y, n):
    h=n//2; q=n//4
    if n==2: return [Y[1][0]]
    C=[]
    for k in range(q):
        f=4*k+1
        C.append(Y[f] if f<=h else (Y[n-f][0], vneg(Y[n-f][1])))
    c=cfft(C,+1)
    o=[None]*h
    for t in range(q):
        z=cmul_w(c[t],t,n,+1)
        o[t]=z[0]; o[t+q]=vneg(z[1])
    return o

def irfft_eo(Y, n):
    h=n//2
    if h==1: e=[Y[0][0]]
    else:
        ee,oo=irfft_eo({k:Y[2*k] for k in range(h//2+1)},h)
        e=[vadd(ee[t],oo[t]) for t in range(h//2)]+[vsub(ee[t],oo[t]) for t in range(h//2)]
    return e, irfft_odd(Y,n)

def comp_F1(u, ld_in, st_tmp, signs, tw=True):
    X=rfft([ld_in(u+4*v) for v in range(16)])
    def put(k,v):
        signs[k]=v.s; st_tmp(k,v.a)
    for f in range(1,8):
        z=cmul_w(X[f],u*f,64) if tw else X[f]
        put((f-1)*8+2*u, z[0]); put((f-1)*8+2*u+1, z[1])
    put(56+u, X[0][0]); put(60+u, X[8][0])

def comp_F2(fs, ld_tmp, st_out, signs, tw=False):
    L=lambda k: V(ld_tmp(k), signs[k])
    for f in fs:
        if f==0:
            r=[L(56+u) for u in range(4)]
            st_out(0, vadd(r[0],r[2]), vadd(r[1],r[3]))
            st_out(16, vsub(r[0],r[2]), vsub(r[3],r[1]))
            s=[L(60+u) for u in range(4)]
            h=np.sqrt(0.5)
            dm=vmul(vsub(s[1],s[3]),h); sn=vmul(vadd(s[1],s[3]),-h)
            st_out(8, vadd(s[0],dm), vsub(sn,s[2]))
            st_out(24, vsub(s[0],dm), vadd(s[2],sn))
        else:
            T=[(L((f-1)*8+2*u),L((f-1)*8+2*u+1)) for u in range(4)]
            if tw: T=[cmul_w(T[u],u*f,64) for u in range(4)]
            s02=cadd(T[0],T[2]); d02=csub(T[0],T[2]); s13=cadd(T[1],T[3])
            d13i=vsub(T[1][1],T[3][1]); e=vsub(T[3][0],T[1][0])
            st_out(f, vadd(s02[0],s13[0]), vadd(s02[1],s13[1]))
            st_out(16+f, vadd(d02[0],d13i), vadd(d02[1],e))
            st_out(32-f, vsub(s02[0],s13[0]), vsub(s13[1],s02[1]))
            st_out(16-f, vsub(d02[0],d13i), vsub(e,d02[1]))

def comp_I1(fs, ld_y, st_tmp):
    for f in fs:
        if f==0:
            yr,yi=V(ld_y(0,0)),V(ld_y(0,1))
            a,b=V(ld_y(16,0)),V(ld_y(16,1))
            for u,v in enumerate((vadd(yr,a),vsub(yi,b),vsub(yr,a),vadd(yi,b))): st_tmp(56+u,out(v))
            Y8=(V(ld_y(8,0)),V(ld_y(8,1))); Y24=(V(ld_y(24,0)),V(ld_y(24,1)))
            h=np.sqrt(0.5)
            p=vsub(Y8[0],Y24[0]); q=vadd(Y8[1],Y24[1])
            p2=vadd(Y8[0],Y24[0]); q2=vsub(Y24[1],Y8[1])
            z0=p2
            z1=vmul(vsub(p,q),h)
            z2=q2
            z3=vmul(vneg(vadd(p,q)),h)
            for u,v in enumerate((z0,z1,z2,z3)): st_tmp(60+u,out(v))
        else:
            def Y(F):
                if F<=32: return (V(ld_y(F,0)),V(ld_y(F,1)))
                return (V(ld_y(64-F,0)),vneg(V(ld_y(64-F,1))))
            G=cfft([Y(f),Y(f+16),Y(f+32),Y(f+48)],+1)
            for u in range(4):
                z=cmul_w(G[u],u*f,64,+1)
                st_tmp((f-1)*8+2*u,out(z[0])); st_tmp((f-1)*8+2*u+1,out(z[1]))

def comp_I2(u, ld_tmp, emit):
    Z={f:(V(ld_tmp((f-1)*8+2*u)),V(ld_tmp((f-1)*8+2*u+1))) for f in range(1,8)}
    Z[0]=(V(ld_tmp(56+u)),None); Z[8]=(V(ld_tmp(60+u)),None)
    e,o=irfft_eo(Z,16)
    for v in range(8):
        emit(u+4*(v+8)-30, vsub(e[v],o[v]))
    if u>=2: emit(u+28-30, vadd(e[7],o[7]))

F32 = jnp.float32
BF16 = jnp.bfloat16
U32 = jnp.uint32

HOP = 34
RANGES = ((0, 7), (7, 15))
XR = 4112
YP = 264
Y_OFF = (0, 96)
RAW_PL = 192
TMP_ANCHOR = 3 * 1024
ZW = 16 * HOP * 8
ZR = 2 * ZW
UNROLLS = dict(x=4, w=4, f=4, g=4, n=16)
FU = 3
FTAIL = 20
CFG = {'x': ((85, 65, 0, 0), 0, 0, -0.5),
       'w': ((135, 65, 0, 0), 3, 1, 0),
       'n': ((100, 70, 50, 90), 0, 0, 0),
       'f': ((110, 80, 45, 100), 0, 4, -1.5),
       'g': ((110, 100, 35, 120), 0, 0, -1.5)}


JITTER = {'x': '44424445555544444424445555535555543444555545444433323203333333332322232333133333333046434444444444445654444344444444355555534233',
          'w': '33322111112112333333222233331331333321334434444444444444441434444444444444444445555444445555535555555555554515566555444455534444',
          'f': '44444542433333333334444446456376666655555555357866764444244444444444444404444444444444443433433333333334444443445553444444444444444424444433302333334322223342222243444444444443455455555554565355557555554444443333333433333333',
          'g': '33424555535666666666666666663355555555444444447444433313313344444444445555554444454331333332332333332333333333444444444444444444444424454434444434444444445555866655555536664666675555354556555555544444244444444455535444333333'}


def x_rows_needed(k):
    if k < 0: return (0, 0)
    last_word = 272 * (RANGES[k][1] - 1) + 2 + 63 + 7 * HOP
    lims = []
    for b in range(2):
        n = 2 * (last_word + 1 - (32 + 2040 * b))
        lims.append(min(4000, max(0, -(-n // 16) * 16)))
    return tuple(lims)


def ds8(x, n=8):
    return pl.ds(pl.multiple_of(x, 8), n)


def interleave(lists, phase=0):
    res, pos = [], [0] * len(lists)
    for _ in range(sum(len(l) for l in lists)):
        j = min((j for j in range(len(lists)) if pos[j] < len(lists[j])),
                key=lambda j: (pos[j] + 0.5 + (phase if j else 0)) / len(lists[j]))
        res.append(lists[j][pos[j]]); pos[j] += 1
    return res


def place(cl, nslot, cw, tail, head, jitter=''):
    cost = [cw[k] for _, k, _ in cl]
    tot, acc, slots, last = max(sum(cost), 1), 0, {}, 0
    for n, (item, c) in enumerate(zip(cl, cost)):
        k = head + (acc * (nslot - tail - head)) // tot + (int(jitter[n]) - 4 if n < len(jitter) else 0)
        last = min(nslot - 1, max(last, k))
        slots.setdefault(last, []).append(item)
        acc += c
    return slots


def _kernel(offs, x_hbm, w_hbm, wo_hbm, o_hbm, xs, *rest):
    Us = rest[:len(RANGES)]
    whA, whB, big, zb, zA, zB, wo, tmp, Tb, sems, xsems, rsems = rest[len(RANGES):]
    whs = (whA, whB)
    bigb = big.bitcast(BF16)
    xsb = xs.bitcast(BF16)
    Uws = tuple(u.bitcast(U32) for u in Us)
    whw = (whA.bitcast(U32), whB.bitcast(U32))
    zw = zb.bitcast(U32)
    zsw = (zA.bitcast(U32), zB.bitcast(U32))
    zs = (zA, zB)
    wow = wo.bitcast(U32)

    def off(k):
        return pl.multiple_of(offs[k], 8)

    def raw_copy(tile, buf):
        col = (tile % 2) * 512 + (tile // 2) * 128
        cs = pl.ds(col, 128) if isinstance(col, int) else pl.ds(pl.multiple_of(col, 128), 128)
        return pltpu.make_async_copy(w_hbm.at[:, :, cs], bigb.at[pl.ds(RAW_PL + 32 * buf, 31), pl.ds(0, 512), :], sems.at[1 + buf])

    def raw_quarter(tile, qd):
        rs = pl.ds(qd * 128, 128) if isinstance(qd, int) else pl.ds(pl.multiple_of(qd * 128, 128), 128)
        return pltpu.make_async_copy(w_hbm.at[:, rs, pl.ds(512 * tile, 128)], bigb.at[pl.ds(RAW_PL + 32 * tile, 31), rs, :],
                                     rsems.at[4 * tile + qd])

    def x_copies(k, ct):
        cs = pl.ds(ct * 128, 128) if isinstance(ct, int) else pl.ds(pl.multiple_of(ct * 128, 128), 128)
        res = []
        for b in range(2):
            lo, hi = x_rows_needed(k - 1)[b], x_rows_needed(k)[b]
            if hi > lo:
                res.append(pltpu.make_async_copy(x_hbm.at[b, pl.ds(lo, hi - lo), cs],
                                                 xsb.at[ct, pl.ds(64 + 4080 * b + lo, hi - lo), :], xsems.at[4 * k + ct]))
        return res

    def x_start(k, ct):
        for c in x_copies(k, ct): c.start()

    def x_wait(k, ct):
        for c in x_copies(k, ct): c.wait()

    def wo_copy(nt):
        return pltpu.make_async_copy(wo_hbm.at[:, pl.ds(nt * 128, 128)], wo.at[nt], sems.at[3])

    first_cuts = (0, 640, 1728, x_rows_needed(0)[0])
    def x_first(j):
        lo, hi = first_cuts[j], first_cuts[j + 1]
        return pltpu.make_async_copy(x_hbm.at[0, pl.ds(lo, hi - lo), pl.ds(0, 128)],
                                     xsb.at[0, pl.ds(64 + lo, hi - lo), :], sems.at[(0, 5, 6)[j]])
    for j in range(3): x_first(j).start()
    x_start(0, 1)
    x_start(0, 2)

    for ct in range(4):
        xs[ct, 0:32, :] = jnp.zeros((32, 128), U32)
        xs[ct, 2032:2072, :] = jnp.zeros((40, 128), U32)
        xs[ct, 4072:4112, :] = jnp.zeros((40, 128), U32)

    def fwd_comps(ld_word, ntaps, st_out, kind):
        p1, signs = [], {}
        for h in range(2):
            def ld_in(n, h=h):
                if n >= ntaps: return None
                return V(pltpu.bitcast(ld_word(n), BF16).astype(F32)[8 * h:8 * h + 8])
            def st_tmp(k, v, h=h): tmp[k * 16 + 8 * h:k * 16 + 8 * h + 8, :] = v
            p1 += [(kind, 0, functools.partial(comp_F1, u, ld_in, st_tmp, signs)) for u in range(4)]
        def ld_tmp(k): return tmp[k * 16:k * 16 + 16, :]
        p2 = [(2, 1, functools.partial(comp_F2, (f,), ld_tmp, st_out, signs)) for f in range(8)]
        return p1, p2

    def x_comps(g, ct, k):
        Ud, gl, rows = Us[k], g - RANGES[k][0], 16 * (RANGES[k][1] - RANGES[k][0])
        def ld_word(n): return xs[ct, pl.ds(272 * g + 2 + n, 8, stride=HOP), :]
        def st_out(f, re, im):
            planes = (re, vsub(re, im) if f == 0 else vadd(re, im), vsub(im, re))
            for p, v in enumerate(planes):
                Ud[f, ct, pl.ds(pl.multiple_of(p * rows + 16 * gl, 16), 16), :] = out(v).astype(BF16)
        return fwd_comps(ld_word, 64, st_out, 4)

    def w_comps(grp, buf, wh):
        def ld_word(t): return big[RAW_PL + 32 * buf + t, ds8(off(2) + 8 * grp), :]
        def st_out(f, re, im):
            for p, v in enumerate((vadd(re, im), im, re)):
                wh[3 * f + p, pl.ds(pl.multiple_of(16 * grp, 16), 16), :] = out(v).astype(BF16)
        return fwd_comps(ld_word, 31, st_out, 1)

    def inv_comps(kind, g, zbase, yb, tmpb, zdst):
        seq = []
        for h in range(2):
            def ld_y(f, p, h=h):
                k1 = big[yb + 3 * f, ds8(off(1) + 16 * g + 8 * h), :]
                k = big[yb + 3 * f + 1 + p, ds8(off(1) + 16 * g + 8 * h), :]
                return k1 - k if p == 0 else k1 + k
            def st_tmp(k, v, h=h): tmp[tmpb + k * 16 + 8 * h:tmpb + k * 16 + 8 * h + 8, :] = v
            def ld_tmp(k, h=h): return tmp[tmpb + k * 16 + 8 * h:tmpb + k * 16 + 8 * h + 8, :]
            if kind == 'f':
                def emit(t, y, h=h):
                    Tb[ds8(t * YP + 16 * g + 8 * h), :] = jnp.tanh(y.a * np.float32(y.s / 32.0)) * np.float32(0.5)
            else:
                def emit(t, y, h=h):
                    th = Tb[ds8(t * YP + 16 * g + 8 * h), :]
                    z = th + th * jnp.tanh(y.a * np.float32(y.s / 64.0))
                    zdst[ds8(zbase + t * 16 + 8 * h), :] = z.astype(BF16)
            seq += [(1, 2, functools.partial(comp_I1, (f,), ld_y, st_tmp)) for f in range(8)]
            seq += [(2, 3, functools.partial(comp_I2, u, ld_tmp, emit)) for u in range(4)]
        return seq

    def run_all(cl):
        for _, _, c in cl: c()

    def xfft_body(g, _, ct):
        p1, p2 = x_comps(g, ct, 0)
        run_all(p1 + p2)
        return 0

    def xfft_ct(ct, _):
        x_wait(0, ct)
        raw_quarter(0, ct - 1).start()
        jax.lax.fori_loop(0, RANGES[0][1], functools.partial(xfft_body, ct=ct), 0)
        return 0

    def xfft_first():
        for j, (g0, g1) in enumerate(((0, 1), (1, 3), (3, RANGES[0][1]))):
            x_first(j).wait()
            if j == 0: x_start(0, 3)
            jax.lax.fori_loop(g0, g1, functools.partial(xfft_body, ct=0), 0)

    def wfft_quarter(qd, _):
        raw_quarter(0, qd).wait()
        @pl.when(qd == 0)
        def _():
            raw_quarter(0, 3).start()
        @pl.when(qd > 0)
        def _():
            x_start(1, qd - 1)
        def body(i, _):
            p1, p2 = w_comps(8 * qd + i, 0, whA)
            run_all(p1 + p2)
            return 0
        jax.lax.fori_loop(0, 8, body, 0)
        return 0

    xfft_first()
    jax.lax.fori_loop(1, 4, xfft_ct, 0)
    jax.lax.fori_loop(0, 4, wfft_quarter, 0)

    def step(variant, par, s, k=None):
        cw, tail, head, mix = CFG[variant]
        UNROLL = UNROLLS[variant]
        NIT = 16 // UNROLL
        wh_cur, wh_nxt = whw[par], whs[1 - par]
        mul = [k] if variant in 'xw' else list(range(len(RANGES)))
        groups = [g for j in mul for g in range(*RANGES[j])]
        if variant in 'fg':
            raw_copy(s + 1, 1 - par).wait()

        def body(i, _):
            streams = []
            if variant == 'x':
                x_wait(k + 1, i)
                @pl.when(i == 0)
                def _():
                    x_start(k + 1, 3)
                raw_quarter(1, i).start()
                seq, prev = [], []
                for g in range(*RANGES[k + 1]):
                    p1, p2 = x_comps(g, i, k + 1)
                    seq += prev + p1
                    prev = p2
                streams.append(seq + prev)
            if variant == 'w':
                raw_quarter(1, i).wait()
            if variant in 'wfg':
                seq, prev = [], []
                for lp in range(2 * UNROLL):
                    p1, p2 = w_comps(2 * UNROLL * i + lp, 1 - par, wh_nxt)
                    seq += prev + p1
                    prev = p2
                streams.append(seq + prev)
            if variant in 'fgn':
                seq = []
                for lp in range(UNROLL):
                    if NIT == 1 and lp == 15: continue
                    g = UNROLL * i + lp
                    seq += inv_comps('g' if variant == 'g' else 'f', g, ((s - 1) // 2) * ZR + g * (HOP * 16),
                                     Y_OFF[1 - par], 2048, zb)
                streams.append(seq)
            slots = place(interleave(streams, mix), 6 * UNROLL * len(groups), cw, tail, head, JITTER.get(variant, ''))
            a_tmp = pl.ds(off(3) + TMP_ANCHOR, 8)
            a_x = pl.ds(off(2) + XR, 8)
            ycur = Y_OFF[par] + i * (6 * UNROLL)
            ak = 0
            for qq in range(2 * UNROLL):
                q = 2 * UNROLL * i + qq
                for m in range(3):
                    parts = []
                    for kt in range(4):
                        rows = []
                        for j in mul:
                            nw = 8 * (RANGES[j][1] - RANGES[j][0])
                            rows.append(pltpu.bitcast(Uws[j][q, kt, pl.ds(m * nw, nw), :], BF16))
                        parts.append(rows[0] if len(rows) == 1 else jnp.concatenate(rows, axis=0))
                    K = jnp.dot(jnp.concatenate(parts, axis=1), pltpu.bitcast(wh_cur[3 * q + m], BF16),
                                preferred_element_type=F32)
                    for j, g in enumerate(groups):
                        piece = K[16 * j:16 * j + 16]
                        big[ycur + 3 * qq + m, ds8(off(0) + 16 * g, 16), :] = piece
                        for kind, _, c in slots.get(ak, ()):
                            if kind == 2: tmp[a_tmp, :] = piece[:8]
                            elif kind == 4: xs[i, a_x, :] = pltpu.bitcast(piece[:8], U32)
                            c()
                        ak += 1
            return 0
        if NIT == 1: body(0, 0)
        else: jax.lax.fori_loop(0, NIT, body, 0)

    for k in range(len(RANGES) - 1):
        step('x', 0, 0, k)
    raw_copy(2, 0).start()
    for nt in range(4): wo_copy(nt).start()
    step('w', 0, 0, len(RANGES) - 1)

    def pair_body(qp, _):
        s = 2 * qp + 1
        @pl.when(s + 2 <= 7)
        def _():
            raw_copy(s + 2, 1).start()
        step('f', 1, s)
        @pl.when(s + 3 <= 7)
        def _():
            raw_copy(s + 3, 0).start()
        step('g', 0, s + 1)
        return 0
    jax.lax.fori_loop(0, 3, pair_body, 0)
    step('n', 1, 7)

    for nt in range(4): wo_copy(nt).wait()

    def out_copy(row0, nrows, b, orow0, nt):
        return pltpu.make_async_copy(xsb.at[nt, pl.ds(row0, nrows), :],
                                     o_hbm.at[b, pl.ds(orow0, nrows), pl.ds(nt * 128, 128)], sems.at[4])
    def pieces(g0, g1):
        res = []
        for b in range(2):
            lo, hi = max(544 * g0, 4080 * b), min(544 * g1, 4080 * b + 4000)
            if hi > lo: res.append((lo, hi - lo, b, lo - 4080 * b))
        return res

    def out_copies(g0, g1, nts=range(4)):
        return [out_copy(a, n, b, o, nt) for nt in nts for (a, n, b, o) in pieces(g0, g1)]

    def fin_chunk(c0, par, with_inv):
        cl = []
        if with_inv:
            for lp in range(FU):
                cl += inv_comps('g', c0 + FU + lp, lp * 544, Y_OFF[1], (lp % 2) * 1024, zs[1 - par])
        slots = place(cl, FU * 4 * HOP, (0, 0, 1, 1), FTAIL, 0)
        a_big = pl.ds(off(4), 8)
        a_tmp = pl.ds(off(3) + TMP_ANCHOR, 8)
        ak = 0
        for lp in range(FU):
            g = c0 + lp
            for nt in range(4):
                gq = g + offs[8 + nt]
                parts = [zw[ds8(kt * ZW + gq * (HOP * 8), HOP * 8), :] for kt in range(3)]
                parts.append(zsw[par][ds8((lp + offs[8 + nt]) * (HOP * 8), HOP * 8), :])
                lhs = jnp.concatenate([pltpu.bitcast(p, BF16) for p in parts], axis=1)
                Rr = jnp.dot(lhs, pltpu.bitcast(wow[nt], BF16), preferred_element_type=F32)
                for t in range(HOP):
                    piece = Rr[16 * t:16 * t + 16]
                    xs[nt, pl.ds(272 * g + t, 8, stride=HOP), :] = pltpu.bitcast(piece.astype(BF16), U32)
                    for kind, _, c in slots.get(ak, ()):
                        if kind == 1: big[RAW_PL + 31, a_big, :] = piece[:8]
                        else: tmp[a_tmp, :] = piece[:8]
                        c()
                    ak += 1
                if not with_inv:
                    for c in out_copies(g, g + 1, (nt,)): c.start()

    def pre_body(g, _):
        run_all(inv_comps('g', g, g * 544, Y_OFF[1], 0, zA))
        return 0
    jax.lax.fori_loop(0, FU, pre_body, 0)
    def fin_pair(j, _):
        for par in range(2):
            fin_chunk(2 * FU * j + par * FU, par, True)
            for jj in range((15 // FU - 1) // 2):
                @pl.when(j == jj)
                def _():
                    c0 = 2 * FU * jj + par * FU
                    for c in out_copies(c0, c0 + FU): c.start()
        return 0
    jax.lax.fori_loop(0, (15 // FU - 1) // 2, fin_pair, 0)
    fin_chunk(15 - FU, 0, False)
    for c0 in range(0, 15 - FU, FU):
        for c in out_copies(c0, c0 + FU): c.wait()
    for g in range(15 - FU, 15):
        for c in out_copies(g, g + 1): c.wait()


def scratch_spec():
    return [
        ('xs', 'vmem', (4, XR + 8, 128), U32),
        *[('U%d' % j, 'vmem', (32, 4, 3 * 16 * (r[1] - r[0]), 128), BF16) for j, r in enumerate(RANGES)],
        ('whA', 'vmem', (96, 512, 128), BF16),
        ('whB', 'vmem', (96, 512, 128), BF16),
        ('big', 'vmem', (RAW_PL + 64, YP, 128), F32),
        ('zb', 'vmem', (3 * ZR, 128), BF16),
        ('zA', 'vmem', (FU * 544, 128), BF16),
        ('zB', 'vmem', (FU * 544, 128), BF16),
        ('wo', 'vmem', (4, 512, 128), BF16),
        ('tmp', 'vmem', (TMP_ANCHOR + 8, 128), F32),
        ('Tb', 'vmem', (34 * YP, 128), F32),
        ('sems', 'sem', 7, None),
        ('xsems', 'sem', 12, None),
        ('rsems', 'sem', 8, None),
    ]


@jax.jit
def pallas_standalone__autoregressive_conv_wavenet__speech_kernel(x, w, w_o):
    B, T, D = x.shape
    offs = jnp.asarray(np.zeros((16,), np.int32))
    return pl.pallas_call(
        _kernel,
        in_specs=[pl.BlockSpec(memory_space=pltpu.SMEM)] + [pl.BlockSpec(memory_space=pl.ANY)] * 3,
        out_specs=pl.BlockSpec(memory_space=pl.ANY),
        out_shape=jax.ShapeDtypeStruct((B, T, D), x.dtype),
        scratch_shapes=[pltpu.SemaphoreType.DMA((sh,)) if kind == 'sem' else pltpu.VMEM(sh, dt)
                        for _, kind, sh, dt in scratch_spec()],
        compiler_params=pltpu.CompilerParams(vmem_limit_bytes=120 * 1024 * 1024),
    )(offs, x, w, w_o)
```
